```python
import os as _os
_os.environ.setdefault("JAX_PLATFORMS", "cpu")
import jax
import jax.numpy as jnp

def _softmax(x, axis=-1):
    return jax.nn.softmax(x, axis=axis)
def _gelu(x):
    return jax.nn.gelu(x, approximate=True)
def _silu(x):
    return jax.nn.silu(x)
def _sigmoid(x):
    return jax.nn.sigmoid(x)
def _layernorm(x, axis=-1, eps=1e-5):
    m = jnp.mean(x, axis=axis, keepdims=True)
    v = jnp.var(x, axis=axis, keepdims=True)
    return (x - m) / jnp.sqrt(v + eps)
def _scatter_add(tgt, idx, src, axis=0):
    return tgt.at[idx].add(src)
def _segment_sum(src, seg, n):
    return jax.ops.segment_sum(src, seg, n)
class _Rng:
    def __init__(self, key):
        self._k = key
    def _next(self):
        self._k, sub = jax.random.split(self._k)
        return sub
    def normal(self, shape):
        return jax.random.normal(self._next(), shape, dtype=jnp.bfloat16)
    def randint(self, lo, hi, shape):
        return jax.random.randint(self._next(), shape, lo, hi, dtype=jnp.int32)
    def uniform(self, shape, lo=0.0, hi=1.0):
        return jax.random.uniform(self._next(), shape, jnp.bfloat16, lo, hi)
    def permutation(self, n):
        return jax.random.permutation(self._next(), n)


kernel_name = 'sequential_preLN__softmax_full_mha__dense_activation_squared_relu__prompt'

def setup_inputs():
    _rng = _Rng(jax.random.key(int.from_bytes(__import__("os").urandom(4), "little")))
    _w = (lambda a: (lambda t: t.astype(jnp.bfloat16) if jnp.issubdtype(t.dtype, jnp.floating) else t)(jnp.asarray(a)))
    def _A_setup():
        B, S, D = 1, 2048, 448
        return {
            "x": _w((lambda *s: _rng.normal(s) * 0.05)(B, S, D)),
            "wqkv": _w((lambda *s: _rng.normal(s) * 0.05)(D, 3 * D)),
            "wo": _w((lambda *s: _rng.normal(s) * 0.05)(D, D)),
        }
    _A_in = _A_setup()

    def _B_setup():
        B, S, D, F = 1, 2048, 448, 1792
        return {
            "x": _w((lambda *s: _rng.normal(s) * 0.05)(B, S, D)),
            "w1": _w((lambda *s: _rng.normal(s) * 0.05)(D, F)),
            "b1": _w((lambda *s: _rng.normal(s) * 0.05)(F)),
            "w2": _w((lambda *s: _rng.normal(s) * 0.05)(F, D)),
            "b2": _w((lambda *s: _rng.normal(s) * 0.05)(D)),
        }
    _B_in = _B_setup()

    return {
        "A_x": _A_in["x"],
        "A_wqkv": _A_in["wqkv"],
        "A_wo": _A_in["wo"],
        "B_x": _B_in["x"],
        "B_w1": _B_in["w1"],
        "B_b1": _B_in["b1"],
        "B_w2": _B_in["w2"],
        "B_b2": _B_in["b2"],
    }

def reference(A_x, A_wqkv, A_wo, B_x, B_w1, B_b1, B_w2, B_b2):
    def _A_ref(x, wqkv, wo):
        B, S, D = x.shape
        H = 16; Dh = D // H
        qkv = (lambda x, *d: x.transpose(*d))((x @ wqkv).reshape(B, S, 3, H, Dh), 2, 0, 3, 1, 4)
        q, k, v = qkv[0], qkv[1], qkv[2]
        scale = Dh ** -0.5
        scores = jnp.einsum("bhqd,bhkd->bhqk", q, k) * scale
        p = _softmax(scores, axis=-1)
        o = jnp.einsum("bhqk,bhkd->bhqd", p, v)
        return (lambda x, *d: x.transpose(*d))(o, 0, 2, 1, 3).reshape(B, S, D) @ wo

    def _B_ref(x, w1, b1, w2, b2):
        h = jnp.einsum("bsd,df->bsf", x, w1) + b1
        zero = jnp.zeros_like(h)
        r = jnp.where(h > zero, h, zero)
        h = r * r
        out = jnp.einsum("bsf,fd->bsd", h, w2) + b2
        return out

    x = A_x
    h = x + _A_ref(_layernorm(x, axis=-1), A_wqkv, A_wo)
    h2 = h + _B_ref(_layernorm(h, axis=-1), B_w1, B_b1, B_w2, B_b2)
    return h2
```

```python
import math

import jax
import jax.numpy as jnp
import jax.experimental.pallas as pl
import jax.experimental.pallas.tpu as pltpu

BF16 = jnp.bfloat16
F32 = jnp.float32
U32 = jnp.uint32

S, D, F, H = 2048, 448, 1792, 16
DH = D // H
DP = 512
BQ = 512
NB = S // BQ
CK = 128
NC = S // CK
G = 4 * DH
EPS = 1e-5
QSCALE = DH ** -0.5 * math.log2(math.e)
QWIN = ((0, 2), (1, 4), (3, 6), (5, 7))
QOFF = (0, 2, 5, 8)

SKEW = 1
F1M = 256
F2K = 256


def _pack(x):
    return pltpu.bitcast(x.astype(BF16), U32)


def _unpack(x):
    return pltpu.bitcast(x, BF16)


def _dot(a, b):
    return jnp.dot(a, b, preferred_element_type=F32)


def _colsum(x):
    r, c = x.shape
    return jnp.sum(jnp.sum(x.reshape(r // 8, 8, c), axis=0), axis=0, keepdims=True)


def _layernorm_t(x):
    d = x - _colsum(x) * (1.0 / D)
    v = _colsum(d * d) * (1.0 / D)
    return d * jax.lax.rsqrt(v + EPS)


def _kernel(x_hbm, wqkv_hbm, wo_hbm, w1_hbm, b1_hbm, w2_hbm, b2_hbm, out_hbm,
            x_s, wqkv_s, wo_s, w1_s, b1_s, w2_s, b2_s, out_s,
            wqkvt_s, wot_s, w1t_s, w2t_s, b2b_s,
            xn_s, q_s, k_s, v_s, s_s, o_s, h_s, g_s, sem_in, sem_out):
    cp_x = [pltpu.make_async_copy(x_hbm.at[:, pl.ds(t * BQ, BQ)], x_s.at[t], sem_in.at[t])
            for t in range(NB)]
    cp_wqkv = pltpu.make_async_copy(wqkv_hbm, wqkv_s, sem_in.at[4])
    cp_rest = [pltpu.make_async_copy(a, b, sem_in.at[5 + i]) for i, (a, b) in enumerate(
        [(wo_hbm, wo_s), (w1_hbm, w1_s), (b1_hbm, b1_s), (w2_hbm, w2_s), (b2_hbm, b2_s)])]
    cp_x[0].start()
    cp_wqkv.start()

    def transpose_w(src, dst, n, extra=None):
        for c in range(pl.cdiv(n, 128)):
            w = min(128, n - c * 128)
            blk = src[:, c * 128:c * 128 + w]
            pad = jnp.zeros((DP - D, w), BF16) if extra is None else extra[:, c * 128:c * 128 + w]
            dst[c * 64:c * 64 + w // 2, :] = pltpu.bitcast(jnp.concatenate([blk, pad], axis=0).T, U32)

    def ln1(t):
        for l in range(BQ // 128):
            ls = slice(l * 128, (l + 1) * 128)
            xn_s[t, 0:D // 2, ls] = _pack(_layernorm_t(x_s[t, :, ls].astype(F32)))
        xn_s[t, D // 2:, :] = jnp.zeros(((DP - D) // 2, BQ), U32)

    row32 = jax.lax.broadcasted_iota(jnp.int32, (32, BQ), 0)

    def qkv(t):
        for part in range(3):
            for g in range(4):
                r0 = part * D + g * G
                y = _dot(_unpack(wqkvt_s[r0 // 2:(r0 + G) // 2, :]), _unpack(xn_s[t]))
                if part == 0:
                    y = y * QSCALE
                    for r, (a, b) in enumerate(QWIN):
                        row = jax.lax.broadcasted_iota(jnp.int32, (16 * (b - a), BQ), 0) + 16 * a
                        keep = (row >= r * DH) & (row < (r + 1) * DH)
                        q_s[t, g, 8 * QOFF[r]:8 * (QOFF[r] + b - a), :] = _pack(
                            jnp.where(keep, y[16 * a:16 * b], 0.0))
                elif part == 1:
                    kt = jnp.concatenate([y.astype(BF16), jnp.zeros((128 - G, BQ), BF16)], axis=0)
                    k_s[g, t * BQ // 2:(t + 1) * BQ // 2, :] = pltpu.bitcast(kt.T, U32)
                else:
                    for r in range(4):
                        lo = r * DH - 4 * (r % 2)
                        ones = (row32 < 4) if r % 2 else (row32 >= DH)
                        v_s[4 * g + r, :, t * BQ:(t + 1) * BQ] = _pack(
                            jnp.where(ones, 1.0, y[lo:lo + 32]))

    cp_x[0].wait()
    for c in cp_x[1:]:
        c.start()
    ln1(0)
    cp_wqkv.wait()
    for c in cp_rest:
        c.start()
    for c in cp_x[1:]:
        c.wait()
    transpose_w(wqkv_s, wqkvt_s, 3 * D)
    for t in range(NB):
        if t + 1 < NB:
            ln1(t + 1)
        if t == 2:
            for c in cp_rest:
                c.wait()
            transpose_w(wo_s, wot_s, D)
            b1 = b1_s[...].astype(F32).reshape(1, F)
            brow = jax.lax.broadcasted_iota(jnp.int32, (DP - D, F), 0)
            transpose_w(w1_s, w1t_s, F, jnp.where(brow == 0, b1, 0.0).astype(BF16))
            w2t_s[...] = pltpu.bitcast(w2_s[...], U32)
            b2 = b2_s[...].astype(F32).reshape(1, D)
            b2b_s[...] = jnp.broadcast_to(b2, (128, D)).T
        qkv(t)

    def block(j, _):
        z = j // NB

        def q_weights(h):
            g, r = divmod(h, 4)
            a, b = QWIN[r]
            parts = [_unpack(q_s[j, g, 8 * QOFF[r]:8 * (QOFF[r] + b - a), :])]
            if a:
                parts.insert(0, jnp.zeros((16 * a, BQ), BF16))
            parts.append(jnp.zeros((128 - 16 * b, BQ), BF16))
            return jnp.concatenate(parts, axis=0)

        st = {}
        NSLOT = NC + SKEW

        def scores(n):
            h, c = divmod(n, NC)
            kk = _unpack(k_s[z + h // 4, c * CK // 2:(c + 1) * CK // 2, :])
            s = _dot(kk, q_weights(h))
            s_s[z + n % NSLOT] = s
            mc = jnp.max(s.reshape(CK // 8, 8, BQ), axis=0)
            st["m"] = mc if c == 0 else jnp.maximum(st["m"], mc)
            if c == NC - 1:
                st["mf", h] = jnp.broadcast_to(jnp.max(st["m"], axis=0, keepdims=True), (8, BQ))

        def probs(n):
            h, c = divmod(n, NC)
            s = s_s[z + n % NSLOT].reshape(CK // 8, 8, BQ)
            st["p"] = jnp.exp2(s - st["mf", h][None]).reshape(CK, BQ).astype(BF16)

        def values(n):
            h, c = divmod(n, NC)
            o = _dot(_unpack(v_s[z + h, :, c * CK:(c + 1) * CK]), st["p"])
            st["acc"] = o if c == 0 else st["acc"] + o
            if c == NC - 1:
                acc = st["acc"]
                lrow = 0 if h % 2 else DH
                o = acc * (1.0 / acc[lrow:lrow + 1])
                base = (h // 2) * 2 * DH
                if h % 2 == 0:
                    o_s[base:base + 24, :] = o[0:24]
                    st["edge"] = o[24:32]
                else:
                    o_s[base + 24:base + 32, :] = jnp.where(row32[0:8] < 4, st["edge"], o[0:8])
                    o_s[base + 32:base + 56, :] = o[8:32]

        HALF = BQ // 2
        KP = 384

        def wo_early(a, m0, m1):
            ls = slice(a * HALF, (a + 1) * HALF)
            y = _dot(_unpack(wot_s[m0 // 2:m1 // 2, 0:KP]), o_s[0:KP, ls].astype(BF16))
            h_s[m0:m1, ls] = y + x_s[j, m0:m1, ls].astype(F32)

        def wo_late(a):
            ls = slice(a * HALF, (a + 1) * HALF)
            rhs = jnp.concatenate([o_s[KP:D, ls].astype(BF16), jnp.zeros((DP - D, HALF), BF16)], axis=0)
            for m0, m1 in ((0, 224), (224, D)):
                y = _dot(_unpack(wot_s[m0 // 2:m1 // 2, KP:DP]), rhs)
                h_s[m0:m1, ls] = h_s[m0:m1, ls] + y

        def ln2(a):
            prow = jax.lax.broadcasted_iota(jnp.int32, (DP - D, 128), 0)
            for l in range(a * HALF // 128, (a + 1) * HALF // 128):
                ls = slice(l * 128, (l + 1) * 128)
                xn_s[z, 0:D // 2, ls] = _pack(_layernorm_t(h_s[:, ls]))
                xn_s[z, D // 2:, ls] = _pack(jnp.where(prow == 0, 1.0, 0.0))

        def ffn1(a):
            ls = slice(a * HALF, (a + 1) * HALF)
            for m in range(0, F, F1M):
                y = _dot(_unpack(w1t_s[m // 2:(m + F1M) // 2, :]), _unpack(xn_s[z, :, ls]))
                y = jnp.where(y > 0, y, 0.0)
                g_s[z, m // 2:(m + F1M) // 2, ls] = _pack(y * y)

        def ffn2(a):
            ls = slice(a * HALF, (a + 1) * HALF)
            y = _dot(_unpack(w2t_s[...]), _unpack(g_s[z, :, ls]))
            b2b = b2b_s[...]
            y = y + h_s[:, ls] + jnp.concatenate([b2b] * (HALF // 128), axis=1)
            out_s[j, :, ls] = y.astype(BF16)

        lag = NC + SKEW
        total = H * NC
        fill = {total + 2: (0, 0, 224), total + 6: (0, 224, D), total + 10: (1, 0, 224)}
        for n in range(total + lag):
            if n >= lag:
                probs(n - lag)
            if n < total:
                scores(n)
            elif n in fill:
                wo_early(*fill[n])
            if n >= lag:
                values(n - lag)
        wo_early(1, 224, D)
        wo_late(0)
        wo_late(1)
        ln2(0)
        ln2(1)
        ffn1(0)
        ffn1(1)
        ffn2(0)
        ffn2(1)
        pltpu.make_async_copy(out_s.at[j], out_hbm.at[:, pl.ds(pl.multiple_of(j * BQ, BQ), BQ)],
                              sem_out.at[j]).start()

    jax.lax.fori_loop(0, NB, block, None)
    for t in range(NB):
        pltpu.make_async_copy(out_s.at[t], out_hbm.at[:, pl.ds(t * BQ, BQ)], sem_out.at[t]).wait()


@jax.jit
def pallas_sequential_preLN__softmax_full_mha__dense_activation_squared_relu__prompt_kernel(A_x, A_wqkv, A_wo, B_x, B_w1, B_b1, B_w2, B_b2):
    del B_x
    hbm = pl.BlockSpec(memory_space=pltpu.HBM)
    vmem = pltpu.VMEM
    out_t = pl.pallas_call(
        _kernel,
        out_shape=jax.ShapeDtypeStruct((D, S), BF16),
        in_specs=[hbm] * 7,
        out_specs=hbm,
        scratch_shapes=[
            vmem((NB, D, BQ), BF16), vmem((D, 3 * D), BF16), vmem((D, D), BF16), vmem((D, F), BF16),
            vmem((F,), BF16), vmem((D, F), BF16), vmem((D,), BF16), vmem((NB, D, BQ), BF16),
            vmem((3 * D // 2, DP), U32), vmem((D // 2, DP), U32), vmem((F // 2, DP), U32),
            vmem((D // 2, F), U32), vmem((D, 128), F32),
            vmem((NB, DP // 2, BQ), U32), vmem((NB, 4, 80, BQ), U32), vmem((4, S // 2, 128), U32),
            vmem((H, 16, S), U32), vmem((NC + SKEW, CK, BQ), F32), vmem((D, BQ), F32),
            vmem((D, BQ), F32), vmem((1, F // 2, BQ), U32),
            pltpu.SemaphoreType.DMA((10,)), pltpu.SemaphoreType.DMA((NB,)),
        ],
        compiler_params=pltpu.CompilerParams(vmem_limit_bytes=100 * 2**20),
    )(A_x[0].T, A_wqkv, A_wo, B_w1, B_b1, B_w2.T, B_b2)
    return out_t.T[None]
```

```python
import math

import jax
import jax.numpy as jnp
import jax.experimental.pallas as pl
import jax.experimental.pallas.tpu as pltpu
import numpy as np

BF16 = jnp.bfloat16
F32 = jnp.float32
U32 = jnp.uint32

S, D, F, H = 2048, 448, 1792, 16
DH = D // H
T = 128
T2 = 2 * T
NP = S // T2
D2, F2 = D // 2, F // 2
NF = F2 // T
G = 4 * DH
EPS = 1e-5
QSCALE = DH ** -0.5 * math.log2(math.e)
QWIN = ((0, 2), (1, 4), (3, 6), (5, 7))
QOFF = (0, 2, 5, 8)
CA, CB, CC = 256, 320, 384

F2M = 112
VP = 6
LAG = NP + 2
NSLOT = 2 * NP
ORDER = list(range(1, VP + 1)) + [0] + list(range(VP + 1, NP))
WQ = (3, 3, 3, 4, 4, 4, 4, 4)
WP = (6, 6)
WS = (16, 16, 15, 16, 16, 16, 16, 16)
MXU_ONLY = (31,)
PO = (2, 1, 0)
TK = 74
TP = 32
LNP = 29
J1 = 10
J2 = 14
PW = 1
FS = 2
WOP = 11
UPR = 3


def _pack(x):
    return pltpu.bitcast(x.astype(BF16), U32)


def _unpack(x):
    return pltpu.bitcast(x, BF16)


def _dot(a, b):
    return jnp.dot(a, b, preferred_element_type=F32)


def _ds(start, size, align):
    return pl.ds(start if isinstance(start, int) else pl.multiple_of(start, align), size)


def _lanes(t, n=1):
    return _ds(t * T, n * T, T)


def _lhs_sums(a11, a12, a21, a22):
    return (a11 + a22, a21 + a22, a11 + a12, a21 - a11, a12 - a22)


def _rhs_terms(b11, b12, b21, b22):
    return (b11 - b22, b11, b22, b11 - b12, b21 - b22, b12 - b22, b21 - b11)


def _strassen(m, top=lambda y: y, bottom=lambda y: y):
    low, m6 = bottom(m(1)), m(6)
    c21 = low + m6
    m0 = m(0)
    c11 = m6 + m0
    c22 = low - m0
    c11 = c11 + m(4)
    c22 = c22 - m(3)
    high = top(m(2))
    c11 = c11 + high
    m5 = m(5)
    return c11, high + m5, c21, c22 + m5


def _weight_tiles(w):
    return (w(0, T), w(T, T2), w(CB, D), jnp.concatenate([w(CA, CB), w(CC, D)], axis=0), w(CA, CC))


def _block_product(sums, tile, rhs, tick=lambda y: y, bias=None):
    def m(i):
        return tick(_dot(sums(i) if i < 5 else tile(i - 5, i - 5), rhs(i)))

    def shared(half):
        def add(y):
            y = y + tick(_dot(tile(half, 2), rhs(7)))
            return y if bias is None else y + bias(half)
        return add

    c = _strassen(m, shared(0), shared(1))
    return [c[2 * half + e] + tick(_dot(tile(half, 3 + e), rhs(8 + e))) for half in range(2) for e in range(2)]


def _store_rhs(dst, z, left, right):
    for m in range(0, T, 16):
        for i, b in enumerate(_rhs_terms(left(m), right(m), left(T + m), right(T + m))):
            dst[z + i, m // 2:m // 2 + 8, :] = _pack(b)
        yield
    for m in range(0, T // 2, 16):
        lb, rc = left(CB + m), right(CC + m)
        halves = ((lb, rc), (left(CA + m), left(CC + m) - rc), (right(CA + m), right(CB + m) - lb))
        for i, pair in enumerate(halves):
            for r, b in zip((m // 2, (T // 2 + m) // 2), pair):
                dst[z + 7 + i, r:r + 8, :] = _pack(b)
        yield


def _run(gen):
    for _ in gen:
        pass


class _Background:
    def __init__(self, ticks, *jobs):
        self.ticks, self.jobs, self.n = ticks, jobs, 0

    def __call__(self, y):
        self.n += 1
        if self.n <= self.ticks:
            for gen, pieces, *marks in self.jobs:
                todo = pieces * self.n // self.ticks - pieces * (self.n - 1) // self.ticks
                for mark in marks if todo else ():
                    mark(y[0:8, 0:T])
                for _ in range(todo):
                    next(gen, None)
                if self.n == self.ticks:
                    _run(gen)
        return y


def _marker(ref, *idx):
    count = [0]
    rows = 8 * 4 // ref.dtype.itemsize

    def mark(v):
        r = count[0] = (count[0] + rows) % ref.shape[-2]
        ref[(*idx, slice(r, r + rows), slice(0, T))] = pltpu.bitcast(v, ref.dtype)
    return mark


def _kernel(x_hbm, wqkv_hbm, wo_hbm, w1_hbm, b1_hbm, w2_hbm, b2_hbm, out_hbm,
            x_s, wqkv_s, wo_s, w1_s, w2_s, out_s, b1_s, b2_s, align_s, b1r_s,
            tqkv_s, to_s, t1_s, aq_s, ak_s, av_s, ao_s, a1_s, a2_s, b2c_s,
            xa_s, xb_s, ob_s, q_s, k_s, v_s, kw_s, kb_s, qb0_s, qb1_s,
            m_s, o_s, h_s, g_s, sem_in, sem_x, sem_w, sem_out, *slots):
    def pair_copy(src, dst, p, sem):
        return pltpu.make_async_copy(src.at[:, _lanes(2 * p, 2)], dst.at[:, _lanes(2 * p, 2)], sem)

    def x_copy(p):
        return pair_copy(x_hbm, x_s, p, sem_x.at[p % 4])

    def mlp_copies(c):
        return [pair_copy(w1_hbm, w1_s, c, sem_w.at[c % 4]), pair_copy(w2_hbm, w2_s, c, sem_w.at[4 + c % 4])]

    cuts = (0, 4 * T, 7 * T, 3 * D)
    cp_wqkv = [pltpu.make_async_copy(wqkv_hbm.at[:, lo:hi], wqkv_s.at[:, lo:hi], sem_w.at[i])
               for i, lo, hi in zip((2, 3, 6), cuts, cuts[1:])]
    cp_wo, cp_b1, cp_b2, cp_align = (
        pltpu.make_async_copy(src, dst, sem_in.at[i])
        for i, (src, dst) in enumerate(((wo_hbm, wo_s), (b1_hbm, b1_s), (b2_hbm, b2_s), (b1_hbm, align_s))))

    def prep_square(src, tiles, sums, part, z):
        for c in range(pl.cdiv(part * D, T), pl.cdiv((part + 1) * D, T)):
            n = min(T, src.shape[1] - c * T)
            for i, w in enumerate(_weight_tiles(lambda lo, hi: src[lo:hi, c * T:c * T + n])):
                tiles[i, c * T // 2:(c * T + n) // 2, :] = _pack(w.T)
            yield
        for m in range(0, D2 // 2, 8):
            rows = (part * D // 2 + m, (part * D + D2) // 2 + m)
            blocks = [_unpack(tiles[i, r:r + 8, :]).astype(F32) for r in rows for i in range(2)]
            for i, a in enumerate(_lhs_sums(*blocks)):
                sums[z + i, m:m + 8, :] = _pack(a)
            yield

    def prep_w1(c, t):
        for e in range(2):
            ls = _lanes(2 * c + e)
            bias = jnp.broadcast_to(b1r_s[0:1, ls], (T, T)).astype(BF16)
            for i, w in enumerate(_weight_tiles(lambda lo, hi: w1_s[lo:hi, ls]) + (bias,)):
                t1_s[c, e, i] = _pack(w.T)
            yield
        for m in range(0, T, 16):
            blocks = [_unpack(t1_s[c, e, i, m // 2:m // 2 + 8, :]).astype(F32) for e in range(2) for i in range(2)]
            for i, a in enumerate(_lhs_sums(*blocks)):
                a1_s[c, i, m:m + 16, :] = a.astype(BF16)
            yield

    def prep_w2(c):
        for m in range(0, D2, 16):
            blocks = [w2_s[r + m:r + m + 16, _lanes(2 * c + e)].astype(F32) for r in (0, D2) for e in range(2)]
            for i, a in enumerate(_lhs_sums(*blocks)):
                a2_s[c, i, m:m + 16, :] = a.astype(BF16)
            yield

    def norm1(p, dst, z):
        count = [0]

        def tile(e):
            def rows(r):
                return x_s[r:r + 16, _lanes(2 * p + e)].astype(F32)

            def mean(f):
                acc = None
                for r in range(0, D, 16):
                    acc = f(rows(r)) if acc is None else acc + f(rows(r))
                    if r % G == G - 16:
                        i, spare = divmod(count[0] % T, T // 2)
                        dst[z + 10 + i, spare:spare + 16, :] = pltpu.bitcast(acc, U32)
                        count[0] += 16
                        yield
                return jnp.sum(acc, axis=0, keepdims=True) * (1.0 / D)

            mu = yield from mean(lambda x: x)
            var = yield from mean(lambda x: (x - mu) * (x - mu))
            scale = jax.lax.rsqrt(var + EPS)
            return lambda r: (rows(r) - mu) * scale

        left = yield from tile(0)
        right = yield from tile(1)
        yield from _store_rhs(dst, z, left, right)

    def qkv(p, xn, z, tick, parts=PO):
        row32 = jax.lax.broadcasted_iota(jnp.int32, (32, T), 0)
        for part in parts:
            for gi in range(2):
                r0 = gi * G // 2
                c = _block_product(
                    lambda i: _unpack((aq_s, ak_s, av_s)[part][z + i, r0:r0 + G // 2, :]),
                    lambda half, i: _unpack(tqkv_s[z + i, pl.ds((part * D + half * D2) // 2 + r0, G // 2), :]),
                    lambda i: _unpack(xn[z + i]), tick)
                for y, g, e in zip(c, (gi, gi, gi + 2, gi + 2), (0, 1, 0, 1)):
                    ls = slice(e * T, (e + 1) * T)
                    if part == 0:
                        words = _pack(y * QSCALE)
                        for r, (lo, hi) in enumerate(QWIN):
                            row = 2 * jax.lax.broadcasted_iota(jnp.int32, (8 * (hi - lo), T), 0) + 16 * lo
                            mine = (row >= r * DH) & (row < (r + 1) * DH)
                            q_s[p, g, 8 * QOFF[r]:8 * (QOFF[r] + hi - lo), ls] = jnp.where(
                                mine, words[8 * lo:8 * hi], np.uint32(0))
                    elif part == 1:
                        k = jnp.concatenate([y, jnp.zeros((T - G, T), F32)], axis=0).astype(BF16).T
                        k_s[g, p, e] = _pack(k)
                        if isinstance(p, int) and p == 0 and e == 0:
                            kw_s[0, g * G // 2:(g + 1) * G // 2, :] = _pack(y)
                    else:
                        for r in range(4):
                            lo = r * DH - 4 * (r % 2)
                            ones = (row32 < 4) if r % 2 else (row32 >= DH)
                            v_s[4 * g + r, p, :, ls] = _pack(jnp.where(ones, 1.0, y[lo:lo + 32]))

    def key_table(c):
        n = D2 // (NP - 1)
        for r in range(n):
            words = kw_s[0, _ds(c * n + r // 8 * 8, 8, 8), :]
            w = jnp.broadcast_to(words[r % 8:r % 8 + 1], (T, T)).T
            for i, v in enumerate((w << 16, w & np.uint32(0xFFFF0000))):
                kb_s[2 * (c * n + r) + i] = pltpu.bitcast(v, F32)
            yield

    def mlp_jobs(c, t, zz):
        return [(prep_w1(c, t), J1, *[_marker(a1_s, zz + NF, t)][:PW]), (prep_w2(c), J2)]

    def table_job(c, zz):
        return key_table(c), TP, _marker(kw_s, zz + 1)

    for cp in (x_copy(0), cp_wqkv[0]):
        cp.start()
    x_copy(0).wait()
    cp_wqkv[1].start()
    _run(norm1(0, xa_s, 0))
    cp_wqkv[2].start()
    cp_wqkv[0].wait()
    x_copy(1).start()
    _run(prep_square(wqkv_s, tqkv_s, aq_s, 0, 0))
    cp_wqkv[1].wait()
    for cp in [cp_b1, cp_align, x_copy(2), x_copy(3)] + mlp_copies(0):
        cp.start()
    qkv(0, xa_s, 0, _Background(26, (prep_square(wqkv_s, tqkv_s, ak_s, 1, 0), 18)), [0])
    cp_wqkv[2].wait()
    x_copy(1).wait()
    qkv(0, xa_s, 0, _Background(22, (prep_square(wqkv_s, tqkv_s, av_s, 2, 0), 18)), [1])
    qkv(0, xa_s, 0, _Background(24, (norm1(1, xb_s, 0), 29)), [2])
    cp_b1.wait()
    cp_align.wait()
    b1r_s[...] = jnp.broadcast_to(b1_s[...].astype(F32).reshape(1, F), (8, F))

    def project(i, _):
        @pl.when(i > 0)
        def _():
            for cp in mlp_copies(2 * i - 1):
                cp.wait()

        for cp in mlp_copies(2 * i) + [x_copy(2 * i + 3)]:
            cp.wait()
        for cp in mlp_copies(2 * i + 1) + mlp_copies(2 * i + 2):
            cp.start()

        @pl.when(i < NP // 2 - 2)
        def _():
            for cp in (x_copy(2 * i + 4), x_copy(2 * i + 5)):
                cp.start()

        @pl.when(i == NP // 2 - 2)
        def _():
            for cp in (cp_wo, cp_b2):
                cp.start()

        x_copy(2 * i + 2).wait()
        z = jax.lax.shift_right_logical(i, 8)
        zz = jax.lax.shift_right_logical(i, 9)
        for e, (cur, nxt) in enumerate(((xb_s, xa_s), (xa_s, xb_s))):
            p = 2 * i + 1 + e
            qkv(p, cur, z, _Background(TK, (norm1(p + 1, nxt, z), LNP, _marker(nxt, zz + 12)),
                                       *mlp_jobs(jnp.maximum(p - 2, 0), e, zz), table_job(p - 1, zz)))
        return z, zz

    z, zz = jax.lax.fori_loop(0, NP // 2 - 1, project, (0, 0))
    for cp in mlp_copies(NF - 2) + mlp_copies(NF - 1) + [cp_wo, cp_b2]:
        cp.wait()
    b2c_s[...] = jnp.broadcast_to(b2_s[...].astype(F32).reshape(1, D), (T, D)).T
    qkv(NP - 1, xb_s, z, _Background(TK, (prep_square(wo_s, to_s, ao_s, 0, z), 18, _marker(ao_s, zz + 5)),
                                     *mlp_jobs(z + NF - 2, 0, zz), *mlp_jobs(z + NF - 1, 1, zz),
                                     table_job(z + NP - 2, zz)))

    work = [(k, l, d) for k in range(0, T, 16) for l in range(2) for d in range(DH)]
    wsum = sum(WS[c] * (sum(WQ[:4] if ORDER[c] == 0 else WQ) + sum(WP) * (c < NP - 1)) for c in range(NP))

    def block(j, _):
        z = jax.lax.shift_right_logical(j, 8)
        zz = jax.lax.shift_right_logical(j, 9)
        st = {}

        def q_window(u):
            a, h = divmod(u, H)
            g, r = divmod(h, 4)
            lo, hi = QWIN[r]
            return _unpack(q_s[2 * j + a, g, 8 * QOFF[r]:8 * (QOFF[r] + hi - lo), :]), lo, hi

        def query_table(u, d0, d1):
            q, lo, _ = q_window(u)
            q = q.astype(F32)
            for d in range(d0, d1):
                r = u % 4 * DH + d - 16 * lo
                (qb0_s, qb1_s)[u % 2][z, d] = jnp.broadcast_to(q[r:r + 1], (8, T2))

        def vpu_scores(n, weight):
            u, c = divmod(n, NP)
            if u in MXU_ONLY:
                return
            first = u % H * DH
            dst = slots[n % NSLOT]
            st["w"] += weight * WS[c]
            upto = len(work) * st["w"] // wsum
            while st["done"] < upto:
                k, l, d0 = work[st["done"]]
                d1 = min(DH, d0 + upto - st["done"])
                ls = slice(l * T, (l + 1) * T)
                prod = (kb_s[first + d0:first + d1, k:k + 16, :].reshape(d1 - d0, 2, 8, T)
                        * (qb0_s, qb1_s)[u % 2][z, d0:d1, :, ls][:, None])
                for d in range(d0, d1):
                    st["sv"] = prod[d - d0] if d == 0 else st["sv"] + prod[d - d0]
                sv = st["sv"]
                if d1 == DH:
                    dst[zz + 1, k:k + 16, ls] = sv.reshape(16, T)
                    st["where", u, k, l] = dst
                    st["m", l] = jnp.maximum(st["m", l], jnp.maximum(sv[0], sv[1]))
                else:
                    r = st["spare"] = (st.get("spare", 0) + 16) % (T - 16)
                    dst[zz + 1, T + r:T + r + 16, ls] = sv.reshape(16, T)
                st["done"] += d1 - d0

        def scores(n):
            u, c = divmod(n, NP)
            p = ORDER[c]
            g = u % H // 4
            q, lo, hi = q_window(u)
            q = jnp.concatenate([jnp.zeros((16 * lo, T2), BF16)] * (lo > 0) + [q]
                                + [jnp.zeros((T - 16 * hi, T2), BF16)], axis=0)
            if p == 0 and u not in MXU_ONLY:
                nk = T // 2
                ss = [_dot(_unpack(k_s[z + g, p, 1, e * nk // 2:(e + 1) * nk // 2, :]), q) for e in range(2)]
            else:
                nk = T
                ss = [_dot(_unpack(k_s[z + g, p, e]), q) for e in range(2)]
            if c == 0:
                st["done"] = st["w"] = 0
            for r in range(0, nk, 8):
                for e in range(2):
                    slots[n % NSLOT][0, e * nk + r:e * nk + r + 8, :] = ss[e][r:r + 8]
                mx = jnp.maximum(ss[0][r:r + 8], ss[1][r:r + 8])
                for l in range(2):
                    ml = mx[:, l * T:(l + 1) * T]
                    st["m", l] = ml if c == 0 and r == 0 else jnp.maximum(st["m", l], ml)
                if r % 16:
                    vpu_scores(n, WQ[r // 16])
            if u + 1 < 2 * H and u + 1 not in MXU_ONLY and 4 * c < DH:
                query_table(u + 1, 4 * c, 4 * c + 4)
            if c == NP - 1:
                m = jnp.concatenate([st["m", 0], st["m", 1]], axis=1)
                m_s[z + u % 2] = jnp.broadcast_to(jnp.max(m, axis=0, keepdims=True), (8, T2))

        def probs(n):
            u, c = divmod(n, NP)
            if c == 0:
                st["max"] = m_s[zz + u % 2]
            if ORDER[c] == 0 and u not in MXU_ONLY:
                s = [jnp.concatenate([st["where", u, k, l][zz + 1, k:k + 16, l * T:(l + 1) * T]
                                      for l in range(2)], axis=1) for k in range(0, T, 16)]
                s = jnp.concatenate(s + [slots[n % NSLOT][0, 0:T, :]], axis=0)
            else:
                s = slots[n % NSLOT][0]
            return jnp.exp2(s.reshape(T2 // 8, 8, T2) - st["max"][None]).reshape(T2, T2).astype(BF16)

        def values(n, p):
            u, c = divmod(n, NP)
            a, h = divmod(u, H)
            y = _dot(_unpack(v_s[z + h, ORDER[c]]), p)
            acc = st["acc"] = y if c == 0 else st["acc"] + y
            if c == NP - 1:
                ones = 0 if h % 2 else DH
                o = acc * (1.0 / acc[ones:ones + 1])
                base = h // 2 * 2 * DH
                if h % 2 == 0:
                    o_s[z + a, base:base + 32, :] = o
                else:
                    row = jax.lax.broadcasted_iota(jnp.int32, (8, T2), 0)
                    edge = o_s[z + a, base + 24:base + 32, :]
                    o_s[z + a, base + 24:base + 32, :] = jnp.where(row < 4, edge, o[0:8])
                    o_s[z + a, base + 32:base + 56, :] = o[8:32]
            return y

        def attention(n, filler=None):
            p = probs(n - LAG) if n >= LAG else None
            if filler is None:
                scores(n)
            else:
                filler()
            y = values(n - LAG, p) if n >= LAG else None
            if filler is None and n % NP < NP - 1 and n // NP not in MXU_ONLY:
                for i, w in enumerate(WP):
                    if y is not None:
                        r = T2 - 16 + 8 * i
                        slots[n % NSLOT][1, r:r + 8, 0:T] = y[16 * i + 8:16 * i + 16, 0:T]
                    vpu_scores(n, w)

        def project_out(a):
            _run(_store_rhs(ob_s, z, *[lambda r, e=e: o_s[z + a, r:r + 16, e * T:(e + 1) * T] for e in range(2)]))
            for m in range(0, D2, G):
                c = _block_product(lambda i: _unpack(ao_s[z + i, m // 2:(m + G) // 2, :]),
                                   lambda half, i: _unpack(to_s[z + i, pl.ds((half * D2 + m) // 2, G // 2), :]),
                                   lambda i: _unpack(ob_s[z + i]))
                for y, r, e in zip(c, (m, m, D2 + m, D2 + m), (0, 1, 0, 1)):
                    h_s[z + a, r:r + G, e * T:(e + 1) * T] = (
                        y + x_s[r:r + G, _lanes(4 * j + 2 * a + e)].astype(F32))

            def norm(e):
                def mean(v):
                    return jnp.sum(jnp.sum(v.reshape(D // 8, 8, T), axis=0), axis=0, keepdims=True) * (1.0 / D)
                x = h_s[z + a, :, e * T:(e + 1) * T]
                d = x - mean(x)
                y = d * jax.lax.rsqrt(mean(d * d) + EPS)
                return lambda r: y[r:r + 16]
            _run(_store_rhs((xa_s, xb_s)[a], z, norm(0), norm(1)))

        def mlp_up(a, t):
            c = _block_product(lambda i: a1_s[z + t, i], lambda half, i: _unpack(t1_s[z + t, half, i]),
                               lambda i: _unpack((xa_s, xb_s)[a][z + i]),
                               bias=lambda half: _unpack(t1_s[z + t, half, 5]).astype(F32))
            c = [jnp.where(y > 0, y, 0.0) for y in c]
            for i, b in enumerate(_rhs_terms(*[y * y for y in c])):
                g_s[z + a, i, t * T // 2:(t + 1) * T // 2, :] = _pack(b)

        def mlp_down(a, m):
            def lhs(i, t):
                if i < 5:
                    return a2_s[z + t, i, m:m + F2M, :]
                return w2_s[pl.ds((i - 5) * D2 + m, F2M), _lanes(2 * t + i - 5)]
            c = _strassen(lambda i: _dot(jnp.concatenate([lhs(i, t) for t in range(NF)], axis=1),
                                         _unpack(g_s[z + a, i])),
                          lambda y: y + b2c_s[m:m + F2M, :], lambda y: y + b2c_s[D2 + m:D2 + m + F2M, :])
            for y, r, e in zip(c, (m, m, D2 + m, D2 + m), (0, 1, 0, 1)):
                y = y + h_s[z + a, r:r + F2M, e * T:(e + 1) * T]
                out_s[r:r + F2M, _lanes(4 * j + 2 * a + e)] = y.astype(BF16)

        total = 2 * H * NP
        query_table(0, 0, DH)
        for n in range(total):
            attention(n)
            if n == total - WOP:
                project_out(0)
        up = list(range(NF))
        for n in range(LAG):
            attention(total + n, (lambda: mlp_up(0, up.pop(0))) if n % FS == 0 and len(up) > UPR else (lambda: None))
        for t in up:
            mlp_up(0, t)
        project_out(1)
        mlp_down(0, 0)
        for t in range(NF):
            mlp_up(1, t)
        for m in range(F2M, D2, F2M):
            mlp_down(0, m)
        pair_copy(out_s, out_hbm, 2 * j, sem_out.at[0]).start()
        for m in range(0, D2, F2M):
            mlp_down(1, m)
            for r in (m, D2 + m):
                pltpu.make_async_copy(out_s.at[r:r + F2M, _lanes(4 * j + 2, 2)],
                                      out_hbm.at[r:r + F2M, _lanes(4 * j + 2, 2)], sem_out.at[0]).start()

    jax.lax.fori_loop(0, NP // 2, block, None)
    pltpu.make_async_copy(out_s, out_hbm, sem_out.at[0]).wait()


@jax.jit
def pallas_sequential_preLN__softmax_full_mha__dense_activation_squared_relu__prompt_kernel(
        A_x, A_wqkv, A_wo, B_x, B_w1, B_b1, B_w2, B_b2):
    del B_x
    hbm = pl.BlockSpec(memory_space=pltpu.HBM)
    vmem = pltpu.VMEM
    dma = pltpu.SemaphoreType.DMA
    out_t = pl.pallas_call(
        _kernel,
        out_shape=jax.ShapeDtypeStruct((D, S), BF16),
        in_specs=[hbm] * 7,
        out_specs=hbm,
        scratch_shapes=[
            vmem((D, S), BF16), vmem((D, 3 * D), BF16), vmem((D, D), BF16), vmem((D, F), BF16),
            vmem((D, F), BF16), vmem((D, S), BF16),
            vmem((F,), BF16), vmem((D,), BF16), vmem((F,), BF16), vmem((8, F), F32),
            vmem((5, 3 * D2, T), U32), vmem((5, D2, T), U32), vmem((NF, 2, 6, T // 2, T), U32),
            *[vmem((6, D2 // 2, T), U32)] * 4, vmem((NF + 1, 5, T, T), BF16), vmem((NF + 1, 5, D2, T), BF16),
            vmem((D, T), F32),
            *[vmem((13, T // 2, T), U32)] * 3,
            vmem((NP, 4, 80, T2), U32), vmem((4, NP, 2, T // 2, T), U32), vmem((H, NP, 16, T2), U32),
            vmem((2, D2, T), U32), vmem((D, T, T), F32), *[vmem((1, DH, 8, T2), F32)] * 2,
            vmem((2, 8, T2), F32), vmem((2, D, T2), F32), vmem((2, D, T2), F32), vmem((2, 7, F2 // 2, T), U32),
            dma((4,)), dma((4,)), dma((8,)), dma((1,)),
            *[vmem((2, T2, T2), F32)] * NSLOT,
        ],
        compiler_params=pltpu.CompilerParams(vmem_limit_bytes=100 * 2**20),
    )(A_x.reshape(S, D).T, A_wqkv, A_wo, B_w1, B_b1, B_w2.T, B_b2)
    return out_t.T.reshape(1, S, D)
```

```python
import math

import jax
import jax.numpy as jnp
import jax.experimental.pallas as pl
import jax.experimental.pallas.tpu as pltpu
import numpy as np

BF16 = jnp.bfloat16
F32 = jnp.float32
U32 = jnp.uint32

S, D, F, H = 2048, 448, 1792, 16
DH = D // H
T = 128
T2 = 2 * T
NP = S // T2
D2, F2 = D // 2, F // 2
NF = F2 // T
G = 4 * DH
EPS = 1e-5
QSCALE = DH ** -0.5 * math.log2(math.e)
QWIN = ((0, 2), (1, 4), (3, 6), (5, 7))
QOFF = (0, 2, 5, 8)
CA, CB, CC = 256, 320, 384

ORDER = (1, 2, 3, 4, 5, 6, 0, 7)
LAG = NP + 2
NSLOT = 2 * NP
STEPS = 2 * H
SHARE = (3, 3, 3, 4, 4, 4, 4, 4, 3, 3)
TABLE_FIRST, TABLE_STEP = 14, 32
TICKS = 70


def _plan_vpu_scores():
    points = [(c, i) for c in range(NP) for i in range(len(SHARE))
              if (c < NP - 1 if i >= 8 else i < 4 or ORDER[c] > 0)]
    work = [(k, l, d) for k in range(0, T, 16) for l in range(2) for d in range(DH)]
    plan, last, done, share = {}, {}, 0, 0
    for c, i in points:
        share += SHARE[i]
        upto = len(work) * share // sum(SHARE[i] for _, i in points)
        plan[c, i] = []
        while done < upto:
            k, l, d0 = work[done]
            d1 = min(DH, d0 + upto - done)
            plan[c, i].append((k, l, d0, d1))
            last[k, l] = c
            done += d1 - d0
    return plan, last


def _pack(x):
    return pltpu.bitcast(x.astype(BF16), U32)


def _unpack(x):
    return pltpu.bitcast(x, BF16)


def _dot(a, b):
    return jnp.dot(a, b, preferred_element_type=F32)


def _lanes(t, n=1):
    return pl.ds(t * T if isinstance(t, int) else pl.multiple_of(t * T, T), n * T)


def _zeros_from(i):
    return jax.lax.shift_right_logical(i, 8), jax.lax.shift_right_logical(i, 9)


def _lhs_sums(a11, a12, a21, a22):
    return (a11 + a22, a21 + a22, a11 + a12, a21 - a11, a12 - a22)


def _rhs_terms(b11, b12, b21, b22):
    return (b11 - b22, b11, b22, b11 - b12, b21 - b22, b12 - b22, b21 - b11)


def _strassen(m, row, own=lambda half, e, y: y):
    low, m6 = row(1, m(1)), m(6)
    c21 = own(1, 0, low + m6)
    m0 = m(0)
    c11 = m6 + m0
    c22 = low - m0
    c22 = own(1, 1, c22 - m(3))
    m5 = m(5)
    c22 = c22 + m5
    high = row(0, m(2))
    c12 = own(0, 1, high + m5)
    return own(0, 0, c11 + high + m(4)), c12, c21, c22


def _weight_pieces(w):
    return (w(0, T), w(T, T2), w(CB, D), jnp.concatenate([w(CA, CB), w(CC, D)], axis=0), w(CA, CC))


def _block_product(sums, piece, rhs, tick=lambda y: y, bias=None):
    def m(i):
        return tick(_dot(sums(i) if i < 5 else piece(i - 5, i - 5), rhs(i)))

    def row(half, y):
        y = y + tick(_dot(piece(half, 2), rhs(7)))
        return y if bias is None else y + bias(half)

    return _strassen(m, row, lambda half, e, y: y + tick(_dot(piece(half, 3 + e), rhs(8 + e))))


def _store_rhs(dst, z, left, right):
    for m in range(0, T, 16):
        for i, b in enumerate(_rhs_terms(left(m), right(m), left(T + m), right(T + m))):
            dst[z + i, m // 2:m // 2 + 8, :] = _pack(b)
        yield
    for m in range(0, T // 2, 16):
        lb, rc = left(CB + m), right(CC + m)
        halves = ((lb, rc), (left(CA + m), left(CC + m) - rc), (right(CA + m), right(CB + m) - lb))
        for i, pair in enumerate(halves):
            for r, b in zip((m // 2, (T // 2 + m) // 2), pair):
                dst[z + 7 + i, r:r + 8, :] = _pack(b)
        yield


def _run(gen):
    for _ in gen:
        pass


class _Background:
    def __init__(self, ticks, *jobs):
        self.ticks, self.jobs, self.n = ticks, jobs, 0

    def __call__(self, y):
        self.n += 1
        if self.n <= self.ticks:
            for gen, pieces, *marks in self.jobs:
                todo = pieces * self.n // self.ticks - pieces * (self.n - 1) // self.ticks
                for mark in marks if todo else ():
                    mark(y[0:8])
                for _ in range(todo):
                    next(gen, None)
                if self.n == self.ticks:
                    _run(gen)
        return y


def _marker(ref, spare):
    count = [0]

    def mark(v):
        r = count[0] = (count[0] + 8) % ref.shape[1]
        ref[spare, r:r + 8, :] = pltpu.bitcast(v, U32)
    return mark


def _kernel(x_hbm, wqkv_hbm, wo_hbm, w1_hbm, b1_hbm, w2_hbm, b2_hbm, out_hbm,
            x_s, wqkv_s, wo_s, w1_s, w2_s, out_s, b1_s, b2_s, align_s, b1r_s,
            tqkv_s, to_s, t1_s, aq_s, ak_s, av_s, ao_s, a1_s, a2_s, b2c_s,
            xa_s, xb_s, ob_s, q_s, k_s, v_s, kw_s, kb_s, qb0_s, qb1_s,
            m_s, o_s, h_s, g_s, sem_in, sem_x, sem_w, sem_out, *slots):
    def pair_copy(src, dst, p, sem):
        return pltpu.make_async_copy(src.at[:, _lanes(2 * p, 2)], dst.at[:, _lanes(2 * p, 2)], sem)

    def x_copy(p):
        return pair_copy(x_hbm, x_s, p, sem_x.at[p % 4])

    def mlp_copies(c):
        return [pair_copy(w1_hbm, w1_s, c, sem_w.at[c % 4]),
                pair_copy(w2_hbm, w2_s, c, sem_w.at[4 + c % 4])]

    cuts = (0, 4 * T, 7 * T, 3 * D)
    cp_wqkv = [pltpu.make_async_copy(wqkv_hbm.at[:, lo:hi], wqkv_s.at[:, lo:hi], sem_w.at[i])
               for i, lo, hi in zip((2, 3, 6), cuts, cuts[1:])]
    cp_wo, cp_b1, cp_b2, cp_align = (
        pltpu.make_async_copy(src, dst, sem_in.at[i]) for i, (src, dst) in enumerate(
            ((wo_hbm, wo_s), (b1_hbm, b1_s), (b2_hbm, b2_s), (b1_hbm, align_s))))

    def prep_square(src, pieces, sums, part, z):
        for c in range(pl.cdiv(part * D, T), pl.cdiv((part + 1) * D, T)):
            n = min(T, src.shape[1] - c * T)
            for i, w in enumerate(_weight_pieces(lambda lo, hi: src[lo:hi, c * T:c * T + n])):
                pieces[i, c * T // 2:(c * T + n) // 2, :] = _pack(w.T)
            yield
        for m in range(0, D2 // 2, 8):
            rows = (part * D // 2 + m, (part * D + D2) // 2 + m)
            blocks = [_unpack(pieces[i, r:r + 8, :]).astype(F32) for r in rows for i in range(2)]
            for i, a in enumerate(_lhs_sums(*blocks)):
                sums[z + i, m:m + 8, :] = _pack(a)
            yield

    def prep_w1(c):
        for e in range(2):
            ls = _lanes(2 * c + e)
            for i in range(5):
                t1_s[c, e, i] = _pack(_weight_pieces(lambda lo, hi: w1_s[lo:hi, ls])[i].T)
            t1_s[c, e, 5] = _pack(jnp.broadcast_to(b1r_s[0:1, ls], (T, T)).astype(BF16).T)
            yield
        for m in range(0, T, 16):
            blocks = [_unpack(t1_s[c, e, i, m // 2:m // 2 + 8, :]).astype(F32)
                      for e in range(2) for i in range(2)]
            for i, a in enumerate(_lhs_sums(*blocks)):
                a1_s[c, i, m:m + 16, :] = a.astype(BF16)
            yield

    def prep_w2(c):
        for m in range(0, D2, 16):
            blocks = [w2_s[r + m:r + m + 16, _lanes(2 * c + e)].astype(F32)
                      for r in (0, D2) for e in range(2)]
            for i, a in enumerate(_lhs_sums(*blocks)):
                a2_s[c, i, m:m + 16, :] = a.astype(BF16)
            yield

    def norm1(p, dst, z):
        count = [0]

        def tile(e):
            def rows(r):
                return x_s[r:r + 16, _lanes(2 * p + e)].astype(F32)

            def mean(f):
                acc = None
                for r in range(0, D, 16):
                    acc = f(rows(r)) if acc is None else acc + f(rows(r))
                    if r % G == G - 16:
                        i, spare = divmod(count[0] % T, T // 2)
                        dst[z + 10 + i, spare:spare + 16, :] = pltpu.bitcast(acc, U32)
                        count[0] += 16
                        yield
                return jnp.sum(acc, axis=0, keepdims=True) * (1.0 / D)

            mu = yield from mean(lambda x: x)
            var = yield from mean(lambda x: (x - mu) * (x - mu))
            scale = jax.lax.rsqrt(var + EPS)
            return lambda r: (rows(r) - mu) * scale

        left = yield from tile(0)
        right = yield from tile(1)
        yield from _store_rhs(dst, z, left, right)

    def put_q(y, p, g, e):
        words = _pack(y * QSCALE)
        for r, (lo, hi) in enumerate(QWIN):
            row = 2 * jax.lax.broadcasted_iota(jnp.int32, (8 * (hi - lo), T), 0) + 16 * lo
            mine = (row >= r * DH) & (row < (r + 1) * DH)
            q_s[p, g, 8 * QOFF[r]:8 * (QOFF[r] + hi - lo), _lanes(e)] = jnp.where(
                mine, words[8 * lo:8 * hi], np.uint32(0))

    def put_k(y, p, g, e):
        k_s[g, p, e] = _pack(jnp.concatenate([y, jnp.zeros((T - G, T), F32)], axis=0).astype(BF16).T)
        if isinstance(p, int) and p == 0 and e == 0:
            kw_s[0, g * G // 2:(g + 1) * G // 2, :] = _pack(y)

    def put_v(y, p, g, e):
        row = jax.lax.broadcasted_iota(jnp.int32, (32, T), 0)
        for r in range(4):
            lo = r * DH - 4 * (r % 2)
            ones = (row < 4) if r % 2 else (row >= DH)
            v_s[4 * g + r, p, :, _lanes(e)] = _pack(jnp.where(ones, 1.0, y[lo:lo + 32]))

    def qkv(p, xn, z, tick, parts=(0, 1, 2)):
        for part in parts:
            for g in range(2):
                r0 = g * G // 2
                c = _block_product(
                    lambda i: _unpack((aq_s, ak_s, av_s)[part][z + i, r0:r0 + G // 2, :]),
                    lambda half, i: _unpack(
                        tqkv_s[z + i, pl.ds((part * D + half * D2) // 2 + r0, G // 2), :]),
                    lambda i: _unpack(xn[z + i]), tick)
                for i, y in enumerate(c):
                    (put_q, put_k, put_v)[part](y, p, g + i // 2 * 2, i % 2)

    def key_table(first, n):
        for r in range(n):
            w = jnp.broadcast_to(kw_s[0, pl.ds(first + r, 1), :], (T, T)).T
            for i, v in enumerate((w << 16, w & np.uint32(0xFFFF0000))):
                kb_s[2 * (first + r) + i] = pltpu.bitcast(v, F32)
            yield

    def mlp_jobs(c):
        return (prep_w1(c), 16), (prep_w2(c), 14)

    for cp in (x_copy(0), cp_wqkv[0]):
        cp.start()
    x_copy(0).wait()
    cp_wqkv[1].start()
    _run(norm1(0, xa_s, 0))
    cp_wqkv[2].start()
    cp_wqkv[0].wait()
    x_copy(1).start()
    _run(prep_square(wqkv_s, tqkv_s, aq_s, 0, 0))
    cp_wqkv[1].wait()
    for cp in [cp_b1, cp_align, x_copy(2), x_copy(3)] + mlp_copies(0):
        cp.start()
    qkv(0, xa_s, 0, _Background(26, (prep_square(wqkv_s, tqkv_s, ak_s, 1, 0), 18)), [0])
    cp_wqkv[2].wait()
    x_copy(1).wait()
    qkv(0, xa_s, 0, _Background(22, (prep_square(wqkv_s, tqkv_s, av_s, 2, 0), 18)), [1])
    qkv(0, xa_s, 0, _Background(24, (norm1(1, xb_s, 0), 29),
                                (key_table(0, TABLE_FIRST), TABLE_FIRST)), [2])
    cp_b1.wait()
    cp_align.wait()
    b1r_s[...] = jnp.broadcast_to(b1_s[...].astype(F32).reshape(1, F), (8, F))

    def project(i, _):
        @pl.when(i > 0)
        def _():
            for cp in mlp_copies(2 * i - 1):
                cp.wait()

        for cp in mlp_copies(2 * i) + [x_copy(2 * i + 3)]:
            cp.wait()
        for cp in mlp_copies(2 * i + 1) + mlp_copies(2 * i + 2):
            cp.start()

        @pl.when(i < NP // 2 - 2)
        def _():
            for cp in (x_copy(2 * i + 4), x_copy(2 * i + 5)):
                cp.start()

        @pl.when(i == NP // 2 - 2)
        def _():
            for cp in (cp_wo, cp_b2):
                cp.start()

        x_copy(2 * i + 2).wait()
        z, zz = _zeros_from(i)
        for e, (cur, nxt) in enumerate(((xb_s, xa_s), (xa_s, xb_s))):
            p = 2 * i + 1 + e
            table = key_table(TABLE_FIRST + (p - 1) * TABLE_STEP, TABLE_STEP)
            qkv(p, cur, z, _Background(
                TICKS, (norm1(p + 1, nxt, z), 29, _marker(nxt, zz + 12)),
                *mlp_jobs(jnp.maximum(p - 2, 0)), (table, TABLE_STEP + 2, _marker(kw_s, zz + 1))))
        return z, zz

    z, zz = jax.lax.fori_loop(0, NP // 2 - 1, project, (0, 0))
    for cp in mlp_copies(NF - 2) + mlp_copies(NF - 1) + [cp_wo, cp_b2]:
        cp.wait()
    b2c_s[...] = jnp.broadcast_to(b2_s[...].astype(F32).reshape(1, D), (T, D)).T
    built = TABLE_FIRST + (NP - 2) * TABLE_STEP
    qkv(NP - 1, xb_s, z, _Background(
        TICKS, (prep_square(wo_s, to_s, ao_s, 0, z), 18, _marker(ao_s, zz + 5)),
        *mlp_jobs(NF - 2), *mlp_jobs(NF - 1),
        (key_table(built, D2 - built), D2 - built + 2, _marker(kw_s, zz + 1))))

    plan, last = _plan_vpu_scores()

    def block(j, _):
        z, zz = _zeros_from(j)
        st = {"spare": 0}

        def uses_vpu(u):
            return u < STEPS - 1

        def q_window(u):
            a, h = divmod(u, H)
            g, r = divmod(h, 4)
            lo, hi = QWIN[r]
            return _unpack(q_s[2 * j + a, g, 8 * QOFF[r]:8 * (QOFF[r] + hi - lo), :]), lo, hi

        def query_table(u, d0, d1):
            q, lo, _ = q_window(u)
            q = q.astype(F32)
            for d in range(d0, d1):
                r = u % 4 * DH + d - 16 * lo
                (qb0_s, qb1_s)[u % 2][z, d] = jnp.broadcast_to(q[r:r + 1], (8, T2))

        def vpu_scores(n, part):
            u, c = divmod(n, NP)
            first = u % H * DH
            for k, l, d0, d1 in plan[c, part]:
                prod = (kb_s[first + d0:first + d1, k:k + 16, :].reshape(d1 - d0, 2, 8, T)
                        * (qb0_s, qb1_s)[u % 2][z, d0:d1, :, _lanes(l)][:, None])
                for d in range(d0, d1):
                    st["sum"] = prod[d - d0] if d == 0 else st["sum"] + prod[d - d0]
                s = st["sum"]
                if d1 < DH:
                    st["spare"] = (st["spare"] + 16) % (T - 16)
                    k = T + st["spare"]
                slots[n % NSLOT][zz + 1, k:k + 16, _lanes(l)] = s.reshape(16, T)
                if d1 == DH:
                    st["max", l] = jnp.maximum(st["max", l], jnp.maximum(s[0], s[1]))

        def scores(n):
            u, c = divmod(n, NP)
            p = ORDER[c]
            g = u % H // 4
            q, lo, hi = q_window(u)
            q = jnp.concatenate([jnp.zeros((16 * lo, T2), BF16)] * (lo > 0) + [q]
                                + [jnp.zeros((T - 16 * hi, T2), BF16)], axis=0)
            if p == 0 and uses_vpu(u):
                nk = T // 2
                ss = [_dot(_unpack(k_s[z + g, p, 1, e * nk // 2:(e + 1) * nk // 2, :]), q)
                      for e in range(2)]
            else:
                nk = T
                ss = [_dot(_unpack(k_s[z + g, p, e]), q) for e in range(2)]
            for r in range(0, nk, 8):
                for e in range(2):
                    slots[n % NSLOT][0, e * nk + r:e * nk + r + 8, :] = ss[e][r:r + 8]
                top = jnp.maximum(ss[0][r:r + 8], ss[1][r:r + 8])
                for l in range(2):
                    t = top[:, l * T:(l + 1) * T]
                    st["max", l] = t if c == 0 and r == 0 else jnp.maximum(st["max", l], t)
                if r % 16 and uses_vpu(u):
                    vpu_scores(n, r // 16)
            if uses_vpu(u + 1) and 4 * c < DH:
                query_table(u + 1, 4 * c, 4 * c + 4)
            if c == NP - 1:
                m = jnp.concatenate([st["max", 0], st["max", 1]], axis=1)
                m_s[z + u % 2] = jnp.broadcast_to(jnp.max(m, axis=0, keepdims=True), (8, T2))

        def probs(n):
            u, c = divmod(n, NP)
            if c == 0:
                st["shift"] = m_s[zz + u % 2]
            if ORDER[c] == 0 and uses_vpu(u):
                s = [jnp.concatenate([slots[u % 2 * NP + last[k, l]][zz + 1, k:k + 16, _lanes(l)]
                                      for l in range(2)], axis=1) for k in range(0, T, 16)]
                s = jnp.concatenate(s + [slots[n % NSLOT][0, 0:T, :]], axis=0)
            else:
                s = slots[n % NSLOT][0]
            p = jnp.exp2(s.reshape(T2 // 8, 8, T2) - st["shift"][None])
            return p.reshape(T2, T2).astype(BF16)

        def values(n, p):
            u, c = divmod(n, NP)
            a, h = divmod(u, H)
            y = _dot(_unpack(v_s[z + h, ORDER[c]]), p)
            acc = st["acc"] = y if c == 0 else st["acc"] + y
            if c == NP - 1:
                ones = 0 if h % 2 else DH
                o = acc * (1.0 / acc[ones:ones + 1])
                base = h // 2 * 2 * DH
                if h % 2 == 0:
                    o_s[z + a, base:base + 32, :] = o
                else:
                    row = jax.lax.broadcasted_iota(jnp.int32, (8, T2), 0)
                    edge = o_s[z + a, base + 24:base + 32, :]
                    o_s[z + a, base + 24:base + 32, :] = jnp.where(row < 4, edge, o[0:8])
                    o_s[z + a, base + 32:base + 56, :] = o[8:32]
            return y

        def project_out(a):
            _run(_store_rhs(ob_s, z, *[lambda r, e=e: o_s[z + a, r:r + 16, _lanes(e)] for e in range(2)]))
            for m in range(0, D2, G):
                c = _block_product(
                    lambda i: _unpack(ao_s[z + i, m // 2:(m + G) // 2, :]),
                    lambda half, i: _unpack(to_s[z + i, pl.ds((half * D2 + m) // 2, G // 2), :]),
                    lambda i: _unpack(ob_s[z + i]))
                for y, r, e in zip(c, (m, m, D2 + m, D2 + m), (0, 1, 0, 1)):
                    x = x_s[r:r + G, _lanes(4 * j + 2 * a + e)]
                    h_s[z + a, r:r + G, _lanes(e)] = y + x.astype(F32)

            def mean(v):
                v = jnp.sum(v.reshape(D // 8, 8, T), axis=0)
                return jnp.sum(v, axis=0, keepdims=True) * (1.0 / D)

            def norm2(e):
                h = h_s[z + a, :, _lanes(e)]
                d = h - mean(h)
                y = d * jax.lax.rsqrt(mean(d * d) + EPS)
                return lambda r: y[r:r + 16]
            _run(_store_rhs((xa_s, xb_s)[a], z, norm2(0), norm2(1)))

        def mlp_up(a, t):
            c = _block_product(lambda i: a1_s[z + t, i], lambda half, i: _unpack(t1_s[z + t, half, i]),
                               lambda i: _unpack((xa_s, xb_s)[a][z + i]),
                               bias=lambda half: _unpack(t1_s[z + t, half, 5]).astype(F32))
            c = [jnp.where(y > 0, y, 0.0) for y in c]
            for i, b in enumerate(_rhs_terms(*[y * y for y in c])):
                g_s[z + a, i, t * T // 2:(t + 1) * T // 2, :] = _pack(b)

        def mlp_down(a, m):
            def lhs(i, t):
                if i < 5:
                    return a2_s[z + t, i, m:m + G, :]
                return w2_s[pl.ds((i - 5) * D2 + m, G), _lanes(2 * t + i - 5)]
            c = _strassen(lambda i: _dot(jnp.concatenate([lhs(i, t) for t in range(NF)], axis=1),
                                         _unpack(g_s[z + a, i])),
                          lambda half, y: y + b2c_s[pl.ds(half * D2 + m, G), :])
            for y, r, e in zip(c, (m, m, D2 + m, D2 + m), (0, 1, 0, 1)):
                y = y + h_s[z + a, r:r + G, _lanes(e)]
                out_s[r:r + G, _lanes(4 * j + 2 * a + e)] = y.astype(BF16)

        total = STEPS * NP
        query_table(0, 0, DH)
        for n in range(total):
            p = probs(n - LAG) if n >= LAG else None
            scores(n)
            y = values(n - LAG, p) if n >= LAG else None
            if n % NP < NP - 1 and uses_vpu(n // NP):
                for i in range(2):
                    if n >= LAG:
                        r = T2 - 16 + 8 * i
                        slots[n % NSLOT][1, r:r + 8, 0:T] = y[16 * i + 8:16 * i + 16, 0:T]
                    vpu_scores(n, 8 + i)
            if n == total - NP - 1:
                project_out(0)
        for n in range(LAG):
            p = probs(total - LAG + n)
            if n % 3 == 0:
                mlp_up(0, n // 3)
            values(total - LAG + n, p)
        for t in range(pl.cdiv(LAG, 3), NF):
            mlp_up(0, t)
        project_out(1)
        mlp_down(0, 0)
        for t in range(NF):
            mlp_up(1, t)
        mlp_down(0, G)
        pair_copy(out_s, out_hbm, 2 * j, sem_out.at[0]).start()
        for m in (0, G):
            mlp_down(1, m)
            for r in (m, D2 + m):
                pltpu.make_async_copy(out_s.at[r:r + G, _lanes(4 * j + 2, 2)],
                                      out_hbm.at[r:r + G, _lanes(4 * j + 2, 2)], sem_out.at[0]).start()

    jax.lax.fori_loop(0, NP // 2, block, None)
    pltpu.make_async_copy(out_s, out_hbm, sem_out.at[0]).wait()


@jax.jit
def pallas_sequential_preLN__softmax_full_mha__dense_activation_squared_relu__prompt_kernel(
        A_x, A_wqkv, A_wo, B_x, B_w1, B_b1, B_w2, B_b2):
    del B_x
    hbm = pl.BlockSpec(memory_space=pltpu.HBM)
    vmem = pltpu.VMEM
    dma = pltpu.SemaphoreType.DMA
    out_t = pl.pallas_call(
        _kernel,
        out_shape=jax.ShapeDtypeStruct((D, S), BF16),
        in_specs=[hbm] * 7,
        out_specs=hbm,
        scratch_shapes=[
            vmem((D, S), BF16), vmem((D, 3 * D), BF16), vmem((D, D), BF16), vmem((D, F), BF16),
            vmem((D, F), BF16), vmem((D, S), BF16),
            vmem((F,), BF16), vmem((D,), BF16), vmem((F,), BF16), vmem((8, F), F32),
            vmem((5, 3 * D2, T), U32), vmem((5, D2, T), U32), vmem((NF, 2, 6, T // 2, T), U32),
            *[vmem((6, D2 // 2, T), U32)] * 4, vmem((NF, 5, T, T), BF16),
            vmem((NF + 1, 5, D2, T), BF16), vmem((D, T), F32),
            *[vmem((13, T // 2, T), U32)] * 3,
            vmem((NP, 4, 80, T2), U32), vmem((4, NP, 2, T // 2, T), U32), vmem((H, NP, 16, T2), U32),
            vmem((2, D2, T), U32), vmem((D, T, T), F32), *[vmem((1, DH, 8, T2), F32)] * 2,
            vmem((2, 8, T2), F32), vmem((2, D, T2), F32), vmem((2, D, T2), F32),
            vmem((2, 7, F2 // 2, T), U32),
            dma((4,)), dma((4,)), dma((8,)), dma((1,)),
            *[vmem((2, T2, T2), F32)] * NSLOT,
        ],
        compiler_params=pltpu.CompilerParams(vmem_limit_bytes=100 * 2**20),
    )(A_x.reshape(S, D).T, A_wqkv, A_wo, B_w1, B_b1, B_w2.T, B_b2)
    return out_t.T.reshape(1, S, D)
```
